```python
import os as _os
_os.environ.setdefault("JAX_PLATFORMS", "cpu")
import jax
import jax.numpy as jnp

def _softmax(x, axis=-1):
    return jax.nn.softmax(x, axis=axis)
def _gelu(x):
    return jax.nn.gelu(x, approximate=True)
def _silu(x):
    return jax.nn.silu(x)
def _sigmoid(x):
    return jax.nn.sigmoid(x)
def _layernorm(x, axis=-1, eps=1e-5):
    m = jnp.mean(x, axis=axis, keepdims=True)
    v = jnp.var(x, axis=axis, keepdims=True)
    return (x - m) / jnp.sqrt(v + eps)
def _scatter_add(tgt, idx, src, axis=0):
    return tgt.at[idx].add(src)
def _segment_sum(src, seg, n):
    return jax.ops.segment_sum(src, seg, n)
class _Rng:
    def __init__(self, key):
        self._k = key
    def _next(self):
        self._k, sub = jax.random.split(self._k)
        return sub
    def normal(self, shape):
        return jax.random.normal(self._next(), shape, dtype=jnp.bfloat16)
    def randint(self, lo, hi, shape):
        return jax.random.randint(self._next(), shape, lo, hi, dtype=jnp.int32)
    def uniform(self, shape, lo=0.0, hi=1.0):
        return jax.random.uniform(self._next(), shape, jnp.bfloat16, lo, hi)
    def permutation(self, n):
        return jax.random.permutation(self._next(), n)


kernel_name = 'parallel_sum__ssm_conv_s5__glu_gated_swiglu__prompt'

def setup_inputs():
    _rng = _Rng(jax.random.key(int.from_bytes(__import__("os").urandom(4), "little")))
    _w = (lambda a: (lambda t: t.astype(jnp.bfloat16) if jnp.issubdtype(t.dtype, jnp.floating) else t)(jnp.asarray(a)))
    def _A_setup():
        B, S, D = 1, 2048, 640
        P = D
        Lambda_re = -0.5 * jnp.exp((lambda *s: _rng.normal(s) * 0.4)(P))
        Lambda_im = (lambda *s: _rng.normal(s) * 0.4)(P) * 1.0
        B_re = (lambda *s: _rng.normal(s) * 0.4)(P, D) * (D ** -0.5)
        B_im = (lambda *s: _rng.normal(s) * 0.4)(P, D) * (D ** -0.5)
        C_re = (lambda *s: _rng.normal(s) * 0.4)(D, P) * (P ** -0.5)
        C_im = (lambda *s: _rng.normal(s) * 0.4)(D, P) * (P ** -0.5)
        log_dt = (lambda *s: _rng.normal(s) * 0.4)(P) * 0.3 - 2.0
        Dskip = (lambda *s: _rng.normal(s) * 0.4)(D)
        return {
            "x": _w((lambda *s: _rng.normal(s) * 0.05)(B, S, D)),
            "Lambda_re": _w(Lambda_re),
            "Lambda_im": _w(Lambda_im),
            "B_re": _w(B_re),
            "B_im": _w(B_im),
            "C_re": _w(C_re),
            "C_im": _w(C_im),
            "log_dt": _w(log_dt),
            "Dskip": _w(Dskip),
        }
    _A_in = _A_setup()

    def _B_setup():
        B, S, D, F = 1, 2048, 640, 1728
        return {
            "x": _w((lambda *s: _rng.normal(s) * 0.05)(B, S, D)),
            "w1": _w((lambda *s: _rng.normal(s) * 0.1)(D, F) * (2.0 / D) ** 0.5),
            "w3": _w((lambda *s: _rng.normal(s) * 0.1)(D, F) * (2.0 / D) ** 0.5),
            "w2": _w((lambda *s: _rng.normal(s) * 0.1)(F, D) * (2.0 / F) ** 0.5),
        }
    _B_in = _B_setup()

    return {
        "A_x": _A_in["x"],
        "A_Lambda_re": _A_in["Lambda_re"],
        "A_Lambda_im": _A_in["Lambda_im"],
        "A_B_re": _A_in["B_re"],
        "A_B_im": _A_in["B_im"],
        "A_C_re": _A_in["C_re"],
        "A_C_im": _A_in["C_im"],
        "A_log_dt": _A_in["log_dt"],
        "A_Dskip": _A_in["Dskip"],
        "B_x": _B_in["x"],
        "B_w1": _B_in["w1"],
        "B_w3": _B_in["w3"],
        "B_w2": _B_in["w2"],
    }

def reference(A_x, A_Lambda_re, A_Lambda_im, A_B_re, A_B_im, A_C_re, A_C_im, A_log_dt, A_Dskip, B_x, B_w1, B_w3, B_w2):
    def _A_ref(x, Lambda_re, Lambda_im, B_re, B_im, C_re, C_im, log_dt, Dskip):
        Bsz, L, H = x.shape
        Lam = Lambda_re + 1j * Lambda_im
        Bmat = B_re + 1j * B_im
        Cmat = C_re + 1j * C_im
        dt = jnp.exp(log_dt)
        Lam_bar = jnp.exp(dt * Lam)
        B_bar = ((Lam_bar - 1.0) / Lam)[:, None] * Bmat
        Bu = jnp.einsum("bld,pd->blp", x + 0j, B_bar)
        h = jnp.zeros_like(Bu[:, 0, :])
        hs = []
        for t in range(L):
            h = Lam_bar[None, :] * h + Bu[:, t, :]
            hs.append(h)
        hseq = jnp.stack(hs, 1)
        y = 2.0 * jnp.einsum("blp,dp->bld", hseq, Cmat).real + x * Dskip[None, None, :]
        return y

    def _B_ref(x, w1, w3, w2):
        gate = jnp.einsum("bsd,df->bsf", x, w1)
        up = jnp.einsum("bsd,df->bsf", x, w3)
        h = _silu(gate) * up
        out = jnp.einsum("bsf,fd->bsd", h, w2)
        return out

    x = A_x
    xn = _layernorm(x, axis=-1)
    return x + _A_ref(xn, A_Lambda_re, A_Lambda_im, A_B_re, A_B_im, A_C_re, A_C_im, A_log_dt, A_Dskip) + _B_ref(xn, B_w1, B_w3, B_w2)
```

```python
import jax
import jax.numpy as jnp
from jax import lax
import jax.experimental.pallas as pl
import jax.experimental.pallas.tpu as pltpu

M = 256
NT = (((1,), (1,)), ((), ()))
LAG = 384
WCH = (256, 384, 512, 512)

def _kernel(x_hbm, lre_hbm, lim_hbm, bre_hbm, bim_hbm, cre_hbm, cim_hbm, ldt_hbm, dsk_hbm,
            w1_hbm, w3_hbm, w2_hbm, o_hbm,
            x_v, vec_v, bre_v, bim_v, cre_v, cim_v, w1_v, w3_v, wt_v, w2_v, xp_ref, op_ref, xb_s, base_s, bu_s, a_s, zero_s, g_s, h_s, y0_s,
            wsem, osem):
    S, D = x_v.shape
    F = w2_v.shape[0]
    FM = w1_v.shape[0]
    FT = F - FM
    T = M // 8
    nl = D // 128
    nb = S // M
    f32 = jnp.float32
    bf16 = jnp.bfloat16

    cps = {}
    def mk(name, src, dst):
        cps[name] = pltpu.make_async_copy(src, dst, wsem.at[len(cps)])
    offs = [sum(WCH[:c]) for c in range(len(WCH))]
    for c, (o, n) in enumerate(zip(offs, WCH)):
        mk(('w1', c), w1_hbm.at[pl.ds(o, n)], w1_v.at[pl.ds(o, n)])
        mk(('w3', c), w3_hbm.at[pl.ds(o, n)], w3_v.at[pl.ds(o, n)])
    for k, v in enumerate((lre_hbm, lim_hbm, ldt_hbm, dsk_hbm)):
        mk(('v', k), v, vec_v[k])
    mk('bre', bre_hbm, bre_v)
    mk('bim', bim_hbm, bim_v)
    mk('t1', w1_hbm.at[pl.ds(FM, FT)], wt_v.at[pl.ds(0, FT)])
    mk('t3', w3_hbm.at[pl.ds(FM, FT)], wt_v.at[pl.ds(FT, FT)])
    mk('w2', w2_hbm, w2_v)
    mk('cre', cre_hbm, cre_v)
    mk('cim', cim_hbm, cim_v)
    mk('x0', x_hbm.at[0, pl.ds(0, M)], x_v.at[pl.ds(0, M)])
    mk('x1', x_hbm.at[0, pl.ds(M, M)], x_v.at[pl.ds(M, M)])
    mk('x2', x_hbm.at[0, pl.ds(2 * M, S - 2 * M)], x_v.at[pl.ds(2 * M, S - 2 * M)])
    def start(*ns):
        for n in ns: cps[n].start()
    def wait(*ns):
        for n in ns: cps[n].wait()
    w = lambda c: (('w1', c), ('w3', c))
    vs = tuple(('v', k) for k in range(4))

    u32 = jnp.uint32
    zero_s[...] = jnp.zeros(zero_s.shape, u32)
    def tie(a, deps):
        t = pltpu.bitcast(a[:16, :128], u32)
        for d in deps:
            t = t | (pltpu.bitcast(d, u32) & zero_s[...])
        top = jnp.concatenate([pltpu.bitcast(t, bf16), a[:16, 128:]], axis=1)
        return jnp.concatenate([top, a[16:]], axis=0)
    lanes = lambda v: [v[:8, l*128:(l+1)*128] for l in range(nl)]

    after = []
    def layernorm(i, npc):
        after.clear()
        xf = x_v[pl.ds(pl.multiple_of(i * M, M), M), :].astype(f32)
        if npc > 1:
            kz = jnp.tile(pltpu.bitcast(h_s[M-16:M, FM-LAG:FM-LAG+128], u32) & zero_s[...], (16, 1))
        for l in range(nl):
            if npc > 1:
                xl = pltpu.bitcast(pltpu.bitcast(x_v[pl.ds(pl.multiple_of(i * M, M), M), l*128:(l+1)*128], u32) | kz, bf16).astype(f32)
            else:
                xl = xf[:, l*128:(l+1)*128]
            xp_ref[l] = xl
        dsk = vec_v[3][...].astype(f32).reshape(1, D)
        tp = T // npc
        for p in range(npc):
            x = jnp.concatenate([jnp.concatenate([xp_ref[l, pl.ds(t, 8, stride=T), :] for t in range(p * tp, (p + 1) * tp)], axis=0) for l in range(nl)], axis=1)
            if npc > 1 and len(after) > 1:
                x = pltpu.bitcast(pltpu.bitcast(x, u32) | jnp.tile(pltpu.bitcast(after[-2], u32) & zero_s[...], (tp, nl)), f32)
            mu = jnp.mean(x, axis=-1, keepdims=True)
            xc = x - mu
            var = jnp.mean(xc * xc, axis=-1, keepdims=True)
            xn = xc * lax.rsqrt(var + 1e-5)
            bs = x + xn * dsk
            xb_s[p * tp * 8:(p + 1) * tp * 8] = xn.astype(bf16)
            base_s[p * tp * 8:(p + 1) * tp * 8] = bs
            yield [bs[t * 8:(t + 1) * 8, -128:] for t in range(tp)]

    def prep():
        lre, lim, ldt = [vec_v[k][...].astype(f32).reshape(1, D) for k in range(3)]
        dt = jnp.exp(ldt)
        mag = jnp.exp(dt * lre)
        ar = mag * jnp.cos(dt * lim); ai = mag * jnp.sin(dt * lim)
        den = lre * lre + lim * lim
        nr = ar - 1.0
        cr = 2.0 * (nr * lre + ai * lim) / den
        ci = 2.0 * (ai * lre - nr * lim) / den
        pr, pi = ar, -ai
        n = 1
        while n < T:
            pr, pi = pr * pr - pi * pi, 2.0 * pr * pi
            n *= 2
        bc = lambda v: jnp.broadcast_to(v, (8, D))
        for l in range(nl):
            sl = slice(l * 128, (l + 1) * 128)
            crc = jnp.broadcast_to(cr[:, sl], (128, 128)).T
            cic = jnp.broadcast_to(ci[:, sl], (128, 128)).T
            dd = []
            for m in range(nl):
                sm = slice(m * 128, (m + 1) * 128)
                br = bre_v[sl, sm].astype(f32); bi = bim_v[sl, sm].astype(f32)
                bre_v[sl, sm] = (crc * br - cic * bi).astype(bf16)
                v = (-(crc * bi + cic * br))
                bim_v[sl, sm] = v.astype(bf16)
                dd.append(v[-8:])
            yield dd
        a_s[0] = bc(ar); a_s[1] = bc(-ai); a_s[2] = bc(pr); a_s[3] = bc(pi)

    def scan(cr, ci, res, per):
        ar, ai = a_s[0], a_s[1]
        step = lambda hr, hi, t: (ar * hr - ai * hi + bu_s[0, t*8:(t+1)*8], ar * hi + ai * hr + bu_s[1, t*8:(t+1)*8])
        hr, hi = bu_s[0, 0:8], bu_s[1, 0:8]
        for t in range(1, T):
            hr, hi = step(hr, hi, t)
            if t % per == per - 1:
                yield lanes(hr) + lanes(hi)
        pr, pi = a_s[2], a_s[3]
        row = lax.broadcasted_iota(jnp.int32, (8, D), 0)
        outr, outi = cr, ci
        for s in range(8):
            er = jnp.broadcast_to(hr[s:s+1], (8, D)); ei = jnp.broadcast_to(hi[s:s+1], (8, D))
            cr, ci = pr * cr - pi * ci + er, pr * ci + pi * cr + ei
            if s < 7:
                outr = jnp.where(row > s, cr, outr); outi = jnp.where(row > s, ci, outi)
        res += [cr, ci]
        hr, hi = outr, outi
        yield lanes(hr) + lanes(hi)
        for t in range(0, T, 2):
            r0, i0 = step(hr, hi, t)
            hr, hi = step(r0, i0, t + 1)
            g_s[0, t*8:(t+2)*8] = jnp.concatenate([r0, hr], axis=0).astype(bf16)
            g_s[1, t*8:(t+2)*8] = jnp.concatenate([i0, hi], axis=0).astype(bf16)
            if t % per == per - 2:
                yield lanes(hr) + lanes(hi)

    def act(g, u):
        return (g * jax.nn.sigmoid(g) * u).astype(bf16)
    def up(xb, c, gen=iter(())):
        for o in range(offs[c], offs[c] + WCH[c], 128):
            xt = tie(xb, next(gen, []))
            g = lax.dot_general(xb, w1_v[pl.ds(o, 128), :], NT, preferred_element_type=f32)
            u = lax.dot_general(xt, w3_v[pl.ds(o, 128), :], NT, preferred_element_type=f32)
            h_s[:, o:o+128] = act(g, u)
    def up_tail(xb):
        gu = lax.dot_general(xb, wt_v[...], NT, preferred_element_type=f32)
        h_s[:, FM:] = act(gu[:, :FT], gu[:, FT:])
    def bu():
        xb = xb_s[...]
        bu_s[0] = lax.dot_general(xb, bre_v[...], NT, preferred_element_type=f32)
        bu_s[1] = lax.dot_general(xb, bim_v[...], NT, preferred_element_type=f32)
    def ocp1(i, l):
        r = pl.ds(pl.multiple_of(i * M, M), M)
        return pltpu.make_async_copy(op_ref.at[l, r], o_hbm.at[0, r, pl.ds(l * 128, 128)], osem.at[i, l])
    ocp = lambda i: [ocp1(i, l) for l in range(nl)]
    col = lambda l: slice(l * 128, (l + 1) * 128)
    def down(l, deps):
        y = jnp.dot(tie(h_s[...], deps), w2_v[:, col(l)], preferred_element_type=f32)
        after.append(y[:8])
        return y
    def out(i, l, y, base, deps=[]):
        y = y + lax.dot_general(tie(g_s[0], deps), cre_v[col(l), :], NT, preferred_element_type=f32)
        y = y + lax.dot_general(g_s[1], cim_v[col(l), :], NT, preferred_element_type=f32)
        y = y + base[:, col(l)]
        after.append(y[:8])
        for t in range(T):
            op_ref[l, pl.ds(i * M + t, 8, stride=T), :] = y[t*8:(t+1)*8]

    start('x0', *vs, *w(0))
    wait('x0', *vs)
    start(*w(1))
    list(layernorm(0, 1))
    xb = xb_s[...]
    wait(*w(0)); start(*w(2))
    up(xb, 0)
    wait(*w(1)); start(*w(3), 't1', 't3', 'bre', 'bim')
    up(xb, 1)
    wait(*w(2)); start('w2')
    up(xb, 2)
    wait(*w(3), 't1', 't3', 'bre', 'bim'); start('cre', 'cim', 'x1')
    pg = prep()
    up_tail(xb)
    up(xb, 3, pg)
    list(pg)
    bu()
    wait('w2')
    z = jnp.zeros((8, D), f32)
    res = []
    sg = scan(z, z, res, 16)
    ys = [down(l, next(sg) if l else []) for l in range(nl)]
    list(sg)
    base = base_s[...]
    for l in range(nl):
        y0_s[l] = ys[l] + base[:, col(l)]
    wait('cre', 'cim', 'x1'); start('x2')
    lg = layernorm(1, 4)
    for l in range(nl):
        out(0, l, y0_s[l], jnp.zeros((M, D), f32), next(lg) if l else [])
    bu()
    wait('x2')

    def body(i, carry, last=False):
        for c in ocp(i - 1): c.start()
        base = base_s[...]
        xb = xb_s[...]
        res = []
        sg = scan(*carry, res, 8)
        up_tail(xb)
        for c in range(len(WCH)):
            up(xb, c, sg)
        list(sg)
        lg = iter(()) if last else layernorm(i + 1, 8)
        for l in range(nl):
            y = down(l, next(lg, []) if l else [])
            out(i, l, y, base, next(lg, []))
            if last:
                ocp1(i, l).start()
        if not last: bu()
        return tuple(res)
    carry = lax.fori_loop(1, nb - 1, body, tuple(res))
    body(nb - 1, carry, True)
    for i in range(nb):
        for c in ocp(i): c.wait()

@jax.jit
def pallas_parallel_sum__ssm_conv_s5__glu_gated_swiglu__prompt_kernel(
    A_x, A_Lambda_re, A_Lambda_im, A_B_re, A_B_im, A_C_re, A_C_im, A_log_dt, A_Dskip, B_x, B_w1, B_w3, B_w2):
    _, S, D = A_x.shape
    F = B_w2.shape[0]
    FM = F // 128 * 128
    bf16 = jnp.bfloat16
    args = (A_x, A_Lambda_re, A_Lambda_im, A_B_re, A_B_im, A_C_re, A_C_im, A_log_dt, A_Dskip, B_w1.T, B_w3.T, B_w2)
    hbm = pl.BlockSpec(memory_space=pltpu.HBM)
    V = pltpu.VMEM
    return pl.pallas_call(
        _kernel,
        in_specs=[hbm] * len(args),
        out_specs=hbm,
        out_shape=jax.ShapeDtypeStruct((1, S, D), jnp.float32),
        scratch_shapes=[V((S, D), bf16), [V((D,), bf16)] * 4, V((D, D), bf16), V((D, D), bf16), V((D, D), bf16), V((D, D), bf16),
                        V((FM, D), bf16), V((FM, D), bf16), V((128, D), bf16), V((F, D), bf16),
                        V((D // 128, M, 128), jnp.float32), V((D // 128, S, 128), jnp.float32),
 V((M, D), bf16), V((M, D), jnp.float32), V((2, M, D), jnp.float32), V((4, 8, D), jnp.float32),
 V((8, 128), jnp.uint32), V((2, M, D), bf16), V((M, F), bf16), V((D // 128, M, 128), jnp.float32),
                        pltpu.SemaphoreType.DMA((24,)), pltpu.SemaphoreType.DMA((S // M, D // 128))],
        compiler_params=pltpu.CompilerParams(vmem_limit_bytes=100 * 1024 * 1024),
    )(*args)
```
